```python
import os as _os
_os.environ.setdefault("JAX_PLATFORMS", "cpu")
import jax
import jax.numpy as jnp

def _softmax(x, axis=-1):
    return jax.nn.softmax(x, axis=axis)
def _gelu(x):
    return jax.nn.gelu(x, approximate=True)
def _silu(x):
    return jax.nn.silu(x)
def _sigmoid(x):
    return jax.nn.sigmoid(x)
def _layernorm(x, axis=-1, eps=1e-5):
    m = jnp.mean(x, axis=axis, keepdims=True)
    v = jnp.var(x, axis=axis, keepdims=True)
    return (x - m) / jnp.sqrt(v + eps)
def _scatter_add(tgt, idx, src, axis=0):
    return tgt.at[idx].add(src)
def _segment_sum(src, seg, n):
    return jax.ops.segment_sum(src, seg, n)
class _Rng:
    def __init__(self, key):
        self._k = key
    def _next(self):
        self._k, sub = jax.random.split(self._k)
        return sub
    def normal(self, shape):
        return jax.random.normal(self._next(), shape, dtype=jnp.bfloat16)
    def randint(self, lo, hi, shape):
        return jax.random.randint(self._next(), shape, lo, hi, dtype=jnp.int32)
    def uniform(self, shape, lo=0.0, hi=1.0):
        return jax.random.uniform(self._next(), shape, jnp.bfloat16, lo, hi)
    def permutation(self, n):
        return jax.random.permutation(self._next(), n)


kernel_name = 'gated_mix__grouped_kv_mqa__ssm_conv_s5__prompt'

def setup_inputs():
    _rng = _Rng(jax.random.key(int.from_bytes(__import__("os").urandom(4), "little")))
    _w = (lambda a: (lambda t: t.astype(jnp.bfloat16) if jnp.issubdtype(t.dtype, jnp.floating) else t)(jnp.asarray(a)))
    def _A_setup():
        B, S, D, H = 1, 2048, 512, 32
        Dh = D // H
        return {
            "x": _w((lambda *s: _rng.normal(s) * 0.05)(B, S, D)),
            "wq": _w((lambda *s: _rng.normal(s) * 1.6)(D, H * Dh)),
            "wk": _w((lambda *s: _rng.normal(s) * 1.6)(D, Dh)),
            "wv": _w((lambda *s: _rng.normal(s) * 0.05)(D, Dh)),
            "wo": _w((lambda *s: _rng.normal(s) * 0.05)(H * Dh, D)),
        }
    _A_in = _A_setup()

    def _B_setup():
        B, S, D = 1, 2048, 512
        P = D
        Lambda_re = -0.5 * jnp.exp((lambda *s: _rng.normal(s) * 0.4)(P))
        Lambda_im = (lambda *s: _rng.normal(s) * 0.4)(P) * 1.0
        B_re = (lambda *s: _rng.normal(s) * 0.4)(P, D) * (D ** -0.5)
        B_im = (lambda *s: _rng.normal(s) * 0.4)(P, D) * (D ** -0.5)
        C_re = (lambda *s: _rng.normal(s) * 0.4)(D, P) * (P ** -0.5)
        C_im = (lambda *s: _rng.normal(s) * 0.4)(D, P) * (P ** -0.5)
        log_dt = (lambda *s: _rng.normal(s) * 0.4)(P) * 0.3 - 2.0
        Dskip = (lambda *s: _rng.normal(s) * 0.4)(D)
        return {
            "x": _w((lambda *s: _rng.normal(s) * 0.05)(B, S, D)),
            "Lambda_re": _w(Lambda_re),
            "Lambda_im": _w(Lambda_im),
            "B_re": _w(B_re),
            "B_im": _w(B_im),
            "C_re": _w(C_re),
            "C_im": _w(C_im),
            "log_dt": _w(log_dt),
            "Dskip": _w(Dskip),
        }
    _B_in = _B_setup()

    return {
        "A_x": _A_in["x"],
        "A_wq": _A_in["wq"],
        "A_wk": _A_in["wk"],
        "A_wv": _A_in["wv"],
        "A_wo": _A_in["wo"],
        "B_x": _B_in["x"],
        "B_Lambda_re": _B_in["Lambda_re"],
        "B_Lambda_im": _B_in["Lambda_im"],
        "B_B_re": _B_in["B_re"],
        "B_B_im": _B_in["B_im"],
        "B_C_re": _B_in["C_re"],
        "B_C_im": _B_in["C_im"],
        "B_log_dt": _B_in["log_dt"],
        "B_Dskip": _B_in["Dskip"],
        "gate_w": _w((lambda *s: _rng.normal(s) * 0.05)(512) * 16.0),
    }

def reference(A_x, A_wq, A_wk, A_wv, A_wo, B_x, B_Lambda_re, B_Lambda_im, B_B_re, B_B_im, B_C_re, B_C_im, B_log_dt, B_Dskip, gate_w):
    def _A_ref(x, wq, wk, wv, wo):
        B, S, D = x.shape
        H = 32
        Dh = D // H
        q = (lambda x, *d: x.transpose(*d))((x @ wq).reshape(B, S, H, Dh), 0, 2, 1, 3)
        k = x @ wk
        v = x @ wv
        scores = jnp.einsum("bhqd,bkd->bhqk", q, k) * (Dh ** -0.5)
        p = _softmax(scores, axis=-1)
        o = jnp.einsum("bhqk,bkd->bhqd", p, v)
        return (lambda x, *d: x.transpose(*d))(o, 0, 2, 1, 3).reshape(B, S, H * Dh) @ wo

    def _B_ref(x, Lambda_re, Lambda_im, B_re, B_im, C_re, C_im, log_dt, Dskip):
        Bsz, L, H = x.shape
        Lam = Lambda_re + 1j * Lambda_im
        Bmat = B_re + 1j * B_im
        Cmat = C_re + 1j * C_im
        dt = jnp.exp(log_dt)
        Lam_bar = jnp.exp(dt * Lam)
        B_bar = ((Lam_bar - 1.0) / Lam)[:, None] * Bmat
        Bu = jnp.einsum("bld,pd->blp", x + 0j, B_bar)
        h = jnp.zeros_like(Bu[:, 0, :])
        hs = []
        for t in range(L):
            h = Lam_bar[None, :] * h + Bu[:, t, :]
            hs.append(h)
        hseq = jnp.stack(hs, 1)
        y = 2.0 * jnp.einsum("blp,dp->bld", hseq, Cmat).real + x * Dskip[None, None, :]
        return y

    x = A_x
    g = _sigmoid((x * gate_w).sum(-1, keepdims=True))
    a = _A_ref(x, A_wq, A_wk, A_wv, A_wo)
    b = _B_ref(x, B_Lambda_re, B_Lambda_im, B_B_re, B_B_im, B_C_re, B_C_im, B_log_dt, B_Dskip)
    return g * a + (1 - g) * b
```

```python
import functools
import jax
import jax.numpy as jnp
import jax.experimental.pallas as pl
import jax.experimental.pallas.tpu as pltpu

f32, bf16 = jnp.float32, jnp.bfloat16

L = 2048
D = 512
H = 32
DH = 16
P = 512
TQ = 512
CK = 128
NCK = L // CK
NSEG = 8
SEG = L // NSEG
NT = (((1,), (1,)), ((), ()))
TN = (((0,), (0,)), ((), ()))
LOG2E = 1.4426950408889634
QK_SCALE = (DH ** -0.5) * LOG2E


def _kernel(x_ref, wq_ref, wk_ref, wv_ref, wo_ref, lre_ref, lim_ref, bre_ref, bim_ref,
            cre_ref, cim_ref, ldt_ref, dsk_ref, gw_ref, out_ref,
            kexp_scr, vt_scr, b_scr, scan_scr, q_scr, s0, s1, m0, m1, o_scr):
    step = pl.program_id(0)

    @pl.when(step == 0)
    def _prologue():
        x = x_ref[...]
        r = jax.lax.broadcasted_iota(jnp.int32, (DH, 128), 0)
        c = jax.lax.broadcasted_iota(jnp.int32, (DH, 128), 1)
        rep = jnp.where((c % DH) == r, 1.0, 0.0).astype(bf16)
        wk_rep = jnp.dot(wk_ref[...], rep, preferred_element_type=f32).astype(bf16)
        k_rep = jnp.dot(x, wk_rep, preferred_element_type=f32) * QK_SCALE
        lane = jax.lax.broadcasted_iota(jnp.int32, (L, 128), 1) // DH
        for j in range(8):
            kexp_scr[j] = jnp.where(lane == j, k_rep, 0.0).astype(bf16)
        vt_scr[...] = jax.lax.dot_general(
            wv_ref[...], x, (((0,), (1,)), ((), ())), preferred_element_type=f32).astype(bf16)

        lam_re = lre_ref[...].astype(f32)
        lam_im = lim_ref[...].astype(f32)
        dt = jnp.exp(ldt_ref[...].astype(f32)).astype(bf16).astype(f32)
        er = jnp.exp(dt * lam_re)
        a_re = er * jnp.cos(dt * lam_im)
        a_im = er * jnp.sin(dt * lam_im)
        nr = a_re - 1.0
        den = lam_re * lam_re + lam_im * lam_im
        c_re = (nr * lam_re + a_im * lam_im) / den
        c_im = (a_im * lam_re - nr * lam_im) / den
        u_re = jax.lax.dot_general(x, bre_ref[...], NT, preferred_element_type=f32)
        u_im = jax.lax.dot_general(x, bim_ref[...], NT, preferred_element_type=f32)
        bu_re = c_re * u_re - c_im * u_im
        bu_im = c_re * u_im + c_im * u_re
        for t in range(4):
            scan_scr[t] = bu_re[:, 128 * t:128 * (t + 1)]
            scan_scr[4 + t] = bu_im[:, 128 * t:128 * (t + 1)]

        ar = [jnp.broadcast_to(a_re[:, 128 * t:128 * (t + 1)], (NSEG, 128)) for t in range(4)]
        ai = [jnp.broadcast_to(a_im[:, 128 * t:128 * (t + 1)], (NSEG, 128)) for t in range(4)]

        def scan_step(b, h, store):
            new = [None] * 8
            for t in range(4):
                hr, hi = h[t], h[4 + t]
                nhr = ar[t] * hr - ai[t] * hi + scan_scr[t, pl.ds(b, NSEG, stride=SEG), :]
                nhi = ar[t] * hi + ai[t] * hr + scan_scr[4 + t, pl.ds(b, NSEG, stride=SEG), :]
                if store:
                    scan_scr[t, pl.ds(b, NSEG, stride=SEG), :] = nhr
                    scan_scr[4 + t, pl.ds(b, NSEG, stride=SEG), :] = nhi
                new[t], new[4 + t] = nhr, nhi
            return tuple(new)

        zero = tuple(jnp.zeros((NSEG, 128), f32) for _ in range(8))
        ends = jax.lax.fori_loop(0, SEG, functools.partial(scan_step, store=False), zero, unroll=4)
        pr, pi = a_re, a_im
        for _ in range(SEG.bit_length() - 1):
            pr, pi = pr * pr - pi * pi, 2.0 * (pr * pi)
        row = jax.lax.broadcasted_iota(jnp.int32, (NSEG, 128), 0)
        init = [None] * 8
        for t in range(4):
            pr_t, pi_t = pr[:, 128 * t:128 * (t + 1)], pi[:, 128 * t:128 * (t + 1)]
            er_t, ei_t = ends[t], ends[4 + t]
            hr, hi = er_t[0:1], ei_t[0:1]
            ir = jnp.zeros((NSEG, 128), f32)
            ii = jnp.zeros((NSEG, 128), f32)
            for s in range(1, NSEG):
                ir = jnp.where(row == s, hr, ir)
                ii = jnp.where(row == s, hi, ii)
                if s < NSEG - 1:
                    hr, hi = (er_t[s:s + 1] + pr_t * hr - pi_t * hi,
                              ei_t[s:s + 1] + pr_t * hi + pi_t * hr)
            init[t], init[4 + t] = ir, ii
        jax.lax.fori_loop(0, SEG, functools.partial(scan_step, store=True), tuple(init), unroll=4)

        h_re = jnp.concatenate([scan_scr[t] for t in range(4)], axis=1).astype(bf16)
        h_im = jnp.concatenate([scan_scr[4 + t] for t in range(4)], axis=1).astype(bf16)
        y = (jax.lax.dot_general(h_re, cre_ref[...], NT, preferred_element_type=f32)
             - jax.lax.dot_general(h_im, cim_ref[...], NT, preferred_element_type=f32))
        xd = (x.astype(f32) * dsk_ref[...].astype(f32)).astype(bf16).astype(f32)
        b_scr[...] = 2.0 * y + xd

    row0 = pl.multiple_of(step * TQ, TQ)
    xt = x_ref[pl.ds(row0, TQ), :]
    q_scr[...] = jnp.dot(xt, wq_ref[...], preferred_element_type=f32).astype(bf16)

    def stage_a(h, s_scr, c, mrun):
        qg = q_scr[:, pl.ds(pl.multiple_of((h // 8) * 128, 128), 128)]
        st = jax.lax.dot_general(kexp_scr[h % 8, c * CK:(c + 1) * CK, :], qg, NT,
                                 preferred_element_type=f32)
        s_scr[c * CK:(c + 1) * CK, :] = st
        mc = jnp.max(st.reshape(CK // 8, 8, TQ), axis=0)
        return mc if mrun is None else jnp.maximum(mrun, mc)

    def stage_b(s_scr, c, m, oacc, lacc):
        p = jnp.exp2(s_scr[c * CK:(c + 1) * CK, :] - m)
        lc = jnp.sum(p.reshape(CK // 8, 8, TQ), axis=0)
        oc = jnp.dot(vt_scr[:, c * CK:(c + 1) * CK], p.astype(bf16), preferred_element_type=f32)
        return (oc if oacc is None else oacc + oc), (lc if lacc is None else lacc + lc)

    def finish_a(m_scr, mrun):
        m_scr[...] = jnp.broadcast_to(jnp.max(mrun, axis=0, keepdims=True), (8, TQ))

    def finish_b(h, oacc, lacc):
        l = jnp.sum(lacc, axis=0, keepdims=True)
        o_scr[pl.ds(pl.multiple_of(h * DH, DH), DH), :] = oacc * (1.0 / l)

    def half(ha, sa, ma, hb, sb, mb):
        m = mb[0:1, :]
        mrun = oacc = lacc = None
        for c in range(NCK):
            if ha is not None:
                mrun = stage_a(ha, sa, c, mrun)
            oacc, lacc = stage_b(sb, c, m, oacc, lacc)
        if ha is not None:
            finish_a(ma, mrun)
        finish_b(hb, oacc, lacc)

    mrun = None
    for c in range(NCK):
        mrun = stage_a(0, s0, c, mrun)
    finish_a(m0, mrun)

    def body(i, carry):
        h = 2 * i
        half(h + 1, s1, m1, h, s0, m0)
        half(h + 2, s0, m0, h + 1, s1, m1)
        return carry

    jax.lax.fori_loop(0, H // 2 - 1, body, 0)
    half(H - 1, s1, m1, H - 2, s0, m0)
    half(None, None, None, H - 1, s1, m1)

    a = jax.lax.dot_general(o_scr[...].astype(bf16), wo_ref[...], TN, preferred_element_type=f32)
    gl = jnp.sum(xt.astype(f32) * gw_ref[...].astype(f32), axis=1, keepdims=True)
    g = jax.nn.sigmoid(gl)
    out_ref[...] = g * a + (1.0 - g) * b_scr[pl.ds(row0, TQ), :]


@jax.jit
def pallas_gated_mix__grouped_kv_mqa__ssm_conv_s5__prompt_kernel(
    A_x: jax.Array,
    A_wq: jax.Array,
    A_wk: jax.Array,
    A_wv: jax.Array,
    A_wo: jax.Array,
    B_x: jax.Array,
    B_Lambda_re: jax.Array,
    B_Lambda_im: jax.Array,
    B_B_re: jax.Array,
    B_B_im: jax.Array,
    B_C_re: jax.Array,
    B_C_im: jax.Array,
    B_log_dt: jax.Array,
    B_Dskip: jax.Array,
    gate_w: jax.Array,
):
    del B_x
    x = A_x.reshape(L, D)
    row = lambda v: v.reshape(1, -1)
    full = lambda shape: pl.BlockSpec(shape, lambda i: (0,) * len(shape))
    operands = (x, A_wq, A_wk, A_wv, A_wo, row(B_Lambda_re), row(B_Lambda_im), B_B_re, B_B_im,
                B_C_re, B_C_im, row(B_log_dt), row(B_Dskip), row(gate_w))
    out = pl.pallas_call(
        _kernel,
        grid=(L // TQ,),
        in_specs=[full(o.shape) for o in operands],
        out_specs=pl.BlockSpec((TQ, D), lambda i: (i, 0)),
        out_shape=jax.ShapeDtypeStruct((L, D), f32),
        scratch_shapes=[
            pltpu.VMEM((8, L, 128), bf16),
            pltpu.VMEM((DH, L), bf16),
            pltpu.VMEM((L, D), f32),
            pltpu.VMEM((8, L, 128), f32),
            pltpu.VMEM((TQ, D), bf16),
            pltpu.VMEM((L, TQ), f32),
            pltpu.VMEM((L, TQ), f32),
            pltpu.VMEM((8, TQ), f32),
            pltpu.VMEM((8, TQ), f32),
            pltpu.VMEM((D, TQ), f32),
        ],
        compiler_params=pltpu.CompilerParams(
            dimension_semantics=("arbitrary",),
            vmem_limit_bytes=100 * 1024 * 1024),
    )(*operands)
    return out.reshape(1, L, D)
```

```python
import jax
import jax.numpy as jnp
import jax.experimental.pallas as pl
import jax.experimental.pallas.tpu as pltpu

f32, bf16 = jnp.float32, jnp.bfloat16

L = 2048
D = 512
H = 32
DH = 16
P = 512
TQ = 512
CK = 128
NCK = L // CK
LAG = 4
NSEG = 8
SEG = L // NSEG
NT = (((1,), (1,)), ((), ()))
TN = (((0,), (0,)), ((), ()))
QK_SCALE = (DH ** -0.5) * 1.4426950408889634


def _kernel(x_ref, wq_ref, wk_ref, wv_ref, wo_ref, lre_ref, lim_ref, bre_ref, bim_ref,
            cre_ref, cim_ref, ldt_ref, dsk_ref, gw_ref, out_ref,
            kexp_scr, vt_scr, y_scr, nat_scr, perm_scr, q_scr, s0, s1, m0, m1, o_scr):
    step = pl.program_id(0)

    @pl.when(step == 0)
    def _prologue():
        x = x_ref[...]
        r = jax.lax.broadcasted_iota(jnp.int32, (DH, 128), 0)
        c = jax.lax.broadcasted_iota(jnp.int32, (DH, 128), 1)
        rep = jnp.where((c % DH) == r, 1.0, 0.0).astype(bf16)
        wk_rep = jnp.dot(wk_ref[...], rep, preferred_element_type=f32).astype(bf16)
        k_rep = jnp.dot(x, wk_rep, preferred_element_type=f32) * QK_SCALE
        lane = jax.lax.broadcasted_iota(jnp.int32, (L, 128), 1) // DH
        for j in range(8):
            kexp_scr[j] = jnp.where(lane == j, k_rep, 0.0).astype(bf16)
        vt_scr[...] = jax.lax.dot_general(
            wv_ref[...], x, (((0,), (1,)), ((), ())), preferred_element_type=f32).astype(bf16)

        lam_re = lre_ref[...].reshape(1, P).astype(f32)
        lam_im = lim_ref[...].reshape(1, P).astype(f32)
        dt = jnp.exp(ldt_ref[...].reshape(1, P).astype(f32)).astype(bf16).astype(f32)
        er = jnp.exp(dt * lam_re)
        a_re = er * jnp.cos(dt * lam_im)
        a_im = er * jnp.sin(dt * lam_im)
        nr = a_re - 1.0
        den = lam_re * lam_re + lam_im * lam_im
        c_re = (nr * lam_re + a_im * lam_im) / den
        c_im = (a_im * lam_re - nr * lam_im) / den
        u_re = jax.lax.dot_general(x, bre_ref[...], NT, preferred_element_type=f32)
        u_im = jax.lax.dot_general(x, bim_ref[...], NT, preferred_element_type=f32)
        bu_re = c_re * u_re - c_im * u_im
        bu_im = c_re * u_im + c_im * u_re
        for t in range(4):
            nat_scr[t] = bu_re[:, 128 * t:128 * (t + 1)]
            nat_scr[4 + t] = bu_im[:, 128 * t:128 * (t + 1)]

        ar = [jnp.broadcast_to(a_re[:, 128 * t:128 * (t + 1)], (NSEG, 128)) for t in range(4)]
        ai = [jnp.broadcast_to(a_im[:, 128 * t:128 * (t + 1)], (NSEG, 128)) for t in range(4)]

        def recur(h, t, br, bi):
            hr, hi = h[t], h[4 + t]
            return ar[t] * hr - ai[t] * hi + br, ar[t] * hi + ai[t] * hr + bi

        def pass1(b, h):
            rows = pl.ds(pl.multiple_of(8 * b, 8), NSEG)
            new = [None] * 8
            for t in range(4):
                br = nat_scr[t, pl.ds(b, NSEG, stride=SEG), :]
                bi = nat_scr[4 + t, pl.ds(b, NSEG, stride=SEG), :]
                perm_scr[t, rows, :] = br
                perm_scr[4 + t, rows, :] = bi
                new[t], new[4 + t] = recur(h, t, br, bi)
            return tuple(new)

        def pass2(b, h):
            rows = pl.ds(pl.multiple_of(8 * b, 8), NSEG)
            new = [None] * 8
            for t in range(4):
                nhr, nhi = recur(h, t, perm_scr[t, rows, :], perm_scr[4 + t, rows, :])
                perm_scr[t, rows, :] = nhr
                perm_scr[4 + t, rows, :] = nhi
                new[t], new[4 + t] = nhr, nhi
            return tuple(new)

        zero = tuple(jnp.zeros((NSEG, 128), f32) for _ in range(8))
        ends = jax.lax.fori_loop(0, SEG, pass1, zero, unroll=16)
        pr, pi = a_re, a_im
        for _ in range(SEG.bit_length() - 1):
            pr, pi = pr * pr - pi * pi, 2.0 * (pr * pi)
        row = jax.lax.broadcasted_iota(jnp.int32, (NSEG, 128), 0)
        init = [None] * 8
        for t in range(4):
            pr_t, pi_t = pr[:, 128 * t:128 * (t + 1)], pi[:, 128 * t:128 * (t + 1)]
            er_t, ei_t = ends[t], ends[4 + t]
            hr, hi = er_t[0:1], ei_t[0:1]
            ir = jnp.zeros((NSEG, 128), f32)
            ii = jnp.zeros((NSEG, 128), f32)
            for s in range(1, NSEG):
                ir = jnp.where(row == s, hr, ir)
                ii = jnp.where(row == s, hi, ii)
                if s < NSEG - 1:
                    hr, hi = (er_t[s:s + 1] + pr_t * hr - pi_t * hi,
                              ei_t[s:s + 1] + pr_t * hi + pi_t * hr)
            init[t], init[4 + t] = ir, ii
        jax.lax.fori_loop(0, SEG, pass2, tuple(init), unroll=16)

        h_re = jnp.concatenate([perm_scr[t] for t in range(4)], axis=1).astype(bf16)
        h_im = jnp.concatenate([perm_scr[4 + t] for t in range(4)], axis=1).astype(bf16)
        y = (jax.lax.dot_general(h_re, cre_ref[...], NT, preferred_element_type=f32)
             - jax.lax.dot_general(h_im, cim_ref[...], NT, preferred_element_type=f32))
        for t in range(4):
            y_scr[t] = 2.0 * y[:, 128 * t:128 * (t + 1)]

    row0 = pl.multiple_of(step * TQ, TQ)
    xt = x_ref[pl.ds(row0, TQ), :]
    q_scr[...] = jnp.dot(xt, wq_ref[...], preferred_element_type=f32).astype(bf16)

    def stage_a(h, s_scr, c, mrun):
        qg = q_scr[:, pl.ds(pl.multiple_of((h // 8) * 128, 128), 128)]
        st = jax.lax.dot_general(kexp_scr[h % 8, c * CK:(c + 1) * CK, :], qg, NT,
                                 preferred_element_type=f32)
        s_scr[c * CK:(c + 1) * CK, :] = st
        mc = jnp.max(st.reshape(CK // 8, 8, TQ), axis=0)
        return mc if mrun is None else jnp.maximum(mrun, mc)

    def stage_b(s_scr, c, m8, oacc, lacc):
        p = jnp.exp2(s_scr[c * CK:(c + 1) * CK, :].reshape(CK // 8, 8, TQ) - m8[None])
        lc = jnp.sum(p, axis=0)
        oc = jnp.dot(vt_scr[:, c * CK:(c + 1) * CK], p.reshape(CK, TQ).astype(bf16),
                     preferred_element_type=f32)
        return (oc if oacc is None else oacc + oc), (lc if lacc is None else lacc + lc)

    def half(ha, sa, ma, hb, sb, mb):
        m8 = mb[...]
        mrun = oacc = lacc = None
        hist = []
        for c in range(NCK):
            if ha is not None:
                mrun = stage_a(ha, sa, c, mrun)
                hist.append(mrun)
            me = m8
            if len(hist) > LAG:
                me = jnp.maximum(m8, jnp.minimum(m8, hist[-1 - LAG]))
            oacc, lacc = stage_b(sb, c, me, oacc, lacc)
        if ha is not None:
            ma[...] = jnp.broadcast_to(jnp.max(mrun, axis=0, keepdims=True), (8, TQ))
        l = jnp.sum(lacc, axis=0, keepdims=True)
        o_scr[pl.ds(pl.multiple_of(hb * DH, DH), DH), :] = oacc * (1.0 / l)

    mrun = None
    for c in range(NCK):
        mrun = stage_a(0, s0, c, mrun)
    m0[...] = jnp.broadcast_to(jnp.max(mrun, axis=0, keepdims=True), (8, TQ))

    def body(i, carry):
        h = 2 * i
        half(h + 1, s1, m1, h, s0, m0)
        half(h + 2, s0, m0, h + 1, s1, m1)
        return carry

    jax.lax.fori_loop(0, H // 2 - 1, body, 0)
    half(H - 1, s1, m1, H - 2, s0, m0)
    half(None, None, None, H - 1, s1, m1)

    a = jax.lax.dot_general(o_scr[...].astype(bf16), wo_ref[...], TN, preferred_element_type=f32)
    xf = xt.astype(f32)
    g = jax.nn.sigmoid(jnp.sum(xf * gw_ref[...].reshape(1, D).astype(f32), axis=1, keepdims=True))
    yb = jnp.concatenate(
        [jnp.concatenate([y_scr[t, pl.ds(2 * step + u, SEG, stride=NSEG), :] for u in range(TQ // SEG)],
                         axis=0) for t in range(4)], axis=1)
    b = yb + (xf * dsk_ref[...].reshape(1, D).astype(f32)).astype(bf16).astype(f32)
    out_ref[...] = g * a + (1.0 - g) * b


@jax.jit
def pallas_gated_mix__grouped_kv_mqa__ssm_conv_s5__prompt_kernel(
    A_x: jax.Array,
    A_wq: jax.Array,
    A_wk: jax.Array,
    A_wv: jax.Array,
    A_wo: jax.Array,
    B_x: jax.Array,
    B_Lambda_re: jax.Array,
    B_Lambda_im: jax.Array,
    B_B_re: jax.Array,
    B_B_im: jax.Array,
    B_C_re: jax.Array,
    B_C_im: jax.Array,
    B_log_dt: jax.Array,
    B_Dskip: jax.Array,
    gate_w: jax.Array,
):
    del B_x
    x = A_x.reshape(L, D)
    full = lambda shape: pl.BlockSpec(shape, lambda i: (0,) * len(shape))
    operands = (x, A_wq, A_wk, A_wv, A_wo, B_Lambda_re, B_Lambda_im, B_B_re, B_B_im,
                B_C_re, B_C_im, B_log_dt, B_Dskip, gate_w)
    out = pl.pallas_call(
        _kernel,
        grid=(L // TQ,),
        in_specs=[full(o.shape) for o in operands],
        out_specs=pl.BlockSpec((TQ, D), lambda i: (i, 0)),
        out_shape=jax.ShapeDtypeStruct((L, D), f32),
        scratch_shapes=[
            pltpu.VMEM((8, L, 128), bf16),
            pltpu.VMEM((DH, L), bf16),
            pltpu.VMEM((4, L, 128), f32),
            pltpu.VMEM((8, L, 128), f32),
            pltpu.VMEM((8, L, 128), f32),
            pltpu.VMEM((TQ, D), bf16),
            pltpu.VMEM((L, TQ), f32),
            pltpu.VMEM((L, TQ), f32),
            pltpu.VMEM((8, TQ), f32),
            pltpu.VMEM((8, TQ), f32),
            pltpu.VMEM((D, TQ), f32),
        ],
        compiler_params=pltpu.CompilerParams(
            dimension_semantics=("arbitrary",),
            vmem_limit_bytes=100 * 1024 * 1024),
    )(*operands)
    return out.reshape(1, L, D)
```
